```python
import jax
import jax.numpy as jnp

def _softmax(x, axis=-1):
    return jax.nn.softmax(x, axis=axis)

def _gelu(x):
    return jax.nn.gelu(x, approximate=True)

def _silu(x):
    return jax.nn.silu(x)

def _sigmoid(x):
    return jax.nn.sigmoid(x)

def _layernorm(x, axis=-1, eps=1e-05):
    m = jnp.mean(x, axis=axis, keepdims=True)
    v = jnp.var(x, axis=axis, keepdims=True)
    return (x - m) / jnp.sqrt(v + eps)

def _scatter_add(tgt, idx, src, axis=0):
    return tgt.at[idx].add(src)

def _segment_sum(src, seg, n):
    return jax.ops.segment_sum(src, seg, n)

class _Rng:

    def __init__(self, key):
        self._k = key

    def _next(self):
        self._k, sub = jax.random.split(self._k)
        return sub

    def normal(self, shape):
        return jax.random.normal(self._next(), shape, dtype=jnp.bfloat16)

    def randint(self, lo, hi, shape):
        return jax.random.randint(self._next(), shape, lo, hi, dtype=jnp.int32)

    def uniform(self, shape, lo=0.0, hi=1.0):
        return jax.random.uniform(self._next(), shape, jnp.bfloat16, lo, hi)

    def permutation(self, n):
        return jax.random.permutation(self._next(), n)
kernel_name = 'adaLN_cond__mha_block_cached__moe_arch_mod__decode'

def setup_inputs():
    _rng = _Rng(jax.random.key(int.from_bytes(__import__("os").urandom(4), "little")))
    _w = lambda a: (lambda t: t.astype(jnp.bfloat16) if jnp.issubdtype(t.dtype, jnp.floating) else t)(jnp.asarray(a))

    def _A_setup():
        B, Sq, D = (4, 1, 448)
        H, Sk, Dh = (16, 16384, 256)
        return {'x': _w((lambda *s: _rng.normal(s) * 0.05)(B, Sq, D)), 'k_cache': _w((lambda *s: _rng.normal(s) * 0.05)(B, H, Sk, Dh)), 'v_cache': _w((lambda *s: _rng.normal(s) * 0.05)(B, H, Sk, Dh)), 'wq': _w((lambda *s: _rng.normal(s) * 0.05)(D, H * Dh) * D ** (-0.5)), 'wo': _w((lambda *s: _rng.normal(s) * 0.05)(H * Dh, D) * (H * Dh) ** (-0.5))}
    _A_in = _A_setup()

    def _B_setup():
        B, S, D, F, C = (4, 1, 448, 1792, 1)
        return {'x': _w((lambda *s: _rng.normal(s) * 0.05)(B, S, D)), 'w_r': _w((lambda *s: _rng.normal(s) * 0.05)(D)), 'w_gate': _w((lambda *s: _rng.normal(s) * 0.05)(D, F)), 'w_up': _w((lambda *s: _rng.normal(s) * 0.05)(D, F)), 'w_down': _w((lambda *s: _rng.normal(s) * 0.05)(F, D))}
    _B_in = _B_setup()
    return {'A_x': _A_in['x'], 'A_k_cache': _A_in['k_cache'], 'A_v_cache': _A_in['v_cache'], 'A_wq': _A_in['wq'], 'A_wo': _A_in['wo'], 'B_x': _B_in['x'], 'B_w_r': _B_in['w_r'], 'B_w_gate': _B_in['w_gate'], 'B_w_up': _B_in['w_up'], 'B_w_down': _B_in['w_down'], 'c': _w((lambda *s: _rng.normal(s) * 0.05)(4, 448)), 'w_mod': _w((lambda *s: _rng.normal(s) * 0.05)(448, 6 * 448) * 448 ** (-0.5))}

def reference(A_x, A_k_cache, A_v_cache, A_wq, A_wo, B_x, B_w_r, B_w_gate, B_w_up, B_w_down, c, w_mod):

    def _A_ref(x, k_cache, v_cache, wq, wo):
        B, Sq, D = x.shape
        H, Dh = (16, 256)
        q = (lambda x, *d: x.transpose(*d))((x @ wq).reshape(B, Sq, H, Dh), 0, 2, 1, 3)
        scores = jnp.einsum('bhqd,bhkd->bhqk', q, k_cache) * Dh ** (-0.5)
        p = _softmax(scores, axis=-1)
        o = jnp.einsum('bhqk,bhkd->bhqd', p, v_cache)
        return (lambda x, *d: x.transpose(*d))(o, 0, 2, 1, 3).reshape(B, Sq, H * Dh) @ wo

    def _B_ref(x, w_r, w_gate, w_up, w_down):
        B, S, D = x.shape
        C = 1
        r = x @ w_r
        idx = jnp.argsort(-r, axis=-1)[:, :C]
        idx_e = jnp.repeat(idx.reshape(B, C, 1), D, axis=2)
        x_sel = jnp.take_along_axis(x, idx_e, axis=1)
        g = _silu(x_sel @ w_gate)
        u = x_sel @ w_up
        y = g * u @ w_down
        r_sel = _sigmoid(jnp.take_along_axis(r, idx, axis=1))
        y = y * r_sel.reshape(B, C, 1)
        b_off = (jnp.arange(B) * S).reshape(B, 1)
        flat_idx = (idx + b_off).reshape(B * C)
        zero = (x * 0.0).reshape(B * S, D)
        upd = _scatter_add(zero, flat_idx, y.reshape(B * C, D), axis=0)
        return x + upd.reshape(B, S, D)
    x = A_x
    mod = (_silu(c) @ w_mod).reshape(c.shape[0], 6, 1, -1)
    sa, ca, ga, sb, cb, gb = (mod[:, 0].copy(), mod[:, 1].copy(), mod[:, 2].copy(), mod[:, 3].copy(), mod[:, 4].copy(), mod[:, 5].copy())
    h = _layernorm(x, axis=-1) * (1 + ca) + sa
    x = x + ga * _A_ref(h, A_k_cache, A_v_cache, A_wq, A_wo)
    h = _layernorm(x, axis=-1) * (1 + cb) + sb
    x = x + gb * _B_ref(h, B_w_r, B_w_gate, B_w_up, B_w_down)
    return x
```

```python
import jax
import jax.numpy as jnp
from jax.experimental import pallas as pl
from jax.experimental.pallas import tpu as pltpu

B, D, H, SK, DH, F = 4, 448, 16, 16384, 256, 1792
F32, BF16 = jnp.float32, jnp.bfloat16
NT_DIMS = (((1,), (1,)), ((), ()))


def _ln(x):
    m = jnp.mean(x, axis=-1, keepdims=True)
    xc = x - m
    v = jnp.mean(xc * xc, axis=-1, keepdims=True)
    return xc / jnp.sqrt(v + 1e-5)


def _silu(x):
    return x * (1.0 / (1.0 + jnp.exp(-x)))


def _make(CK=1024, NBUF=4, SUB=64, WSUB=32, ffn_last=True, wo_last=False):
    NC = SK // CK
    NU = B * H
    NT = NU * NC
    SPLIT = CK // SUB

    def kernel(x_hbm, k_hbm, v_hbm, wq_hbm, wot_hbm, wr_hbm, wg_hbm, wu_hbm, wdt_hbm, c_hbm, wmod_hbm, o_ref,
               kbuf, vbuf, ksem, vsem, wq_v, wot_v, wg_v, wu_v, wdt_v, wmod_v, x_v, c_v, wr_v, wsem, q_scr):
        def start(t, slot):
            base = t * CK
            for j in range(SPLIT):
                pltpu.make_async_copy(k_hbm.at[pl.ds(base + j * SUB, SUB)], kbuf.at[slot, pl.ds(j * SUB, SUB)], ksem.at[slot]).start(priority=0)
                pltpu.make_async_copy(v_hbm.at[pl.ds(base + j * SUB, SUB)], vbuf.at[slot, pl.ds(j * SUB, SUB)], vsem.at[slot]).start(priority=1)

        def wait_k(slot):
            pltpu.make_async_copy(kbuf.at[slot], kbuf.at[slot], ksem.at[slot]).wait()

        def wait_v(slot):
            pltpu.make_async_copy(vbuf.at[slot], vbuf.at[slot], vsem.at[slot]).wait()

        W = dict(x=(x_hbm, x_v, 0), c=(c_hbm, c_v, 1), wr=(wr_hbm, wr_v, 2), wmod=(wmod_hbm, wmod_v, 3), wq=(wq_hbm, wq_v, 4),
                 wo=(wot_hbm, wot_v, 5), wg=(wg_hbm, wg_v, 6), wu=(wu_hbm, wu_v, 7), wd=(wdt_hbm, wdt_v, 8))

        def wstart(name):
            s, d, i = W[name]
            if len(s.shape) == 2 and s.shape[0] == D:
                for j in range(D // WSUB):
                    pltpu.make_async_copy(s.at[pl.ds(j * WSUB, WSUB)], d.at[pl.ds(j * WSUB, WSUB)], wsem.at[i]).start(priority=j % 2)
            else:
                pltpu.make_async_copy(s, d, wsem.at[i]).start()

        def wwait(name):
            s, d, i = W[name]
            pltpu.make_async_copy(d, d, wsem.at[i]).wait()

        for n in ("x", "c", "wr", "wmod", "wq"):
            wstart(n)
        for j in range(NBUF - 1):
            start(j, j)
        if not wo_last:
            wstart("wo")
        if not ffn_last:
            wstart("wg"); wstart("wu"); wstart("wd")

        wwait("x"); wwait("c"); wwait("wr")
        zpad = jnp.zeros((8 - B, D), F32)
        x8 = jnp.concatenate([x_v[...].astype(F32), zpad], axis=0)
        c8 = jnp.concatenate([c_v[...].astype(F32), zpad], axis=0)
        sc = _silu(c8).astype(BF16)
        ln1 = _ln(x8)
        wwait("wmod")
        mod = jnp.dot(sc, wmod_v[...], preferred_element_type=F32)
        sa, ca, ga, sb, cb, gb = [mod[:, i * D:(i + 1) * D] for i in range(6)]
        h1 = (ln1 * (1.0 + ca) + sa).astype(BF16)
        wwait("wq")
        q = jnp.dot(h1, wq_v[...], preferred_element_type=F32).astype(BF16).astype(F32) * (DH ** -0.5)
        for h in range(H):
            q_scr[h] = q[:, h * DH:(h + 1) * DH]
        if not wo_last:
            wwait("wo")
        row = jax.lax.broadcasted_iota(jnp.int32, (8, DH), 0)

        def attend(b, h):
            u = b * H + h
            qb = jnp.broadcast_to(q_scr[h, pl.ds(b, 1), :], (8, DH)).astype(BF16)

            def step(c, carry):
                m, l, acc = carry
                t = u * NC + c
                slot = t % NBUF
                nxt = t + NBUF - 1

                @pl.when(nxt < NT)
                def _():
                    start(nxt, nxt % NBUF)

                if ffn_last:
                    @pl.when(nxt == NT - 1)
                    def _():
                        wstart("wg"); wstart("wu"); wstart("wd")
                wait_k(slot)
                wait_v(slot)
                s = jax.lax.dot_general(qb, kbuf[slot], NT_DIMS, preferred_element_type=F32)
                m_new = jnp.maximum(m, jnp.max(s, axis=1, keepdims=True))
                alpha = jnp.exp(m - m_new)
                p = jnp.exp(s - m_new)
                l = alpha * l + jnp.sum(p, axis=1, keepdims=True)
                acc = alpha * acc + jnp.dot(p.astype(BF16), vbuf[slot], preferred_element_type=F32)
                return m_new, l, acc

            m, l, acc = jax.lax.fori_loop(0, NC, step, (jnp.full((8, 1), -jnp.inf, F32), jnp.zeros((8, 1), F32), jnp.zeros((8, DH), F32)))
            return jnp.where(row == b, acc / l, 0.0).astype(BF16)

        attn = jnp.zeros((8, D), F32)

        def bloop(b, attn):
            for h in range(H):
                o = attend(b, h)
                attn = attn + jax.lax.dot_general(o, wot_v[:, h * DH:(h + 1) * DH], NT_DIMS, preferred_element_type=F32)
            return attn
        attn = jax.lax.fori_loop(0, B, bloop, attn)

        x1 = x8 + ga * attn
        h2 = _ln(x1) * (1.0 + cb) + sb
        h2b = h2.astype(BF16)
        r = jnp.sum(h2b.astype(F32) * wr_v[...].astype(F32).reshape(1, D), axis=-1, keepdims=True)
        rs = 1.0 / (1.0 + jnp.exp(-r))
        wwait("wg")
        g = jnp.dot(h2b, wg_v[...], preferred_element_type=F32)
        wwait("wu")
        up = jnp.dot(h2b, wu_v[...], preferred_element_type=F32)
        a = (_silu(g) * up).astype(BF16)
        wwait("wd")
        y = jax.lax.dot_general(a, wdt_v[...], NT_DIMS, preferred_element_type=F32) * rs
        out = x1 + gb * (h2 + (h2 * 0.0 + y))
        o_ref[...] = out[0:B].astype(BF16)

    hbm = pl.BlockSpec(memory_space=pltpu.HBM)
    f = pl.pallas_call(
        kernel,
        out_shape=jax.ShapeDtypeStruct((B, D), BF16),
        in_specs=[hbm] * 11,
        out_specs=pl.BlockSpec(memory_space=pltpu.VMEM),
        scratch_shapes=[
            pltpu.VMEM((NBUF, CK, DH), BF16), pltpu.VMEM((NBUF, CK, DH), BF16),
            pltpu.SemaphoreType.DMA((NBUF,)), pltpu.SemaphoreType.DMA((NBUF,)),
            pltpu.VMEM((D, H * DH), BF16), pltpu.VMEM((D, H * DH), BF16),
            pltpu.VMEM((D, F), BF16), pltpu.VMEM((D, F), BF16), pltpu.VMEM((D, F), BF16),
            pltpu.VMEM((D, 6 * D), BF16), pltpu.VMEM((B, D), BF16), pltpu.VMEM((B, D), BF16), pltpu.VMEM((D,), BF16),
            pltpu.SemaphoreType.DMA((9,)),
            pltpu.VMEM((H, 8, DH), F32),
        ],
        compiler_params=pltpu.CompilerParams(vmem_limit_bytes=100 * 1024 * 1024),
    )

    def run(A_x, A_k_cache, A_v_cache, A_wq, A_wo, B_x, B_w_r, B_w_gate, B_w_up, B_w_down, c, w_mod):
        out = f(A_x.reshape(B, D), A_k_cache.reshape(B * H * SK, DH), A_v_cache.reshape(B * H * SK, DH), A_wq, A_wo.T, B_w_r, B_w_gate, B_w_up, B_w_down.T, c, w_mod)
        return out.reshape(B, 1, D)
    return run


@jax.jit
def pallas_adaLN_cond__mha_block_cached__moe_arch_mod__decode_kernel(
    A_x, A_k_cache, A_v_cache, A_wq, A_wo, B_x, B_w_r, B_w_gate, B_w_up, B_w_down, c, w_mod,
):
    return _make()(A_x, A_k_cache, A_v_cache, A_wq, A_wo, B_x, B_w_r, B_w_gate, B_w_up, B_w_down, c, w_mod)
```

```python
import jax
import jax.numpy as jnp
from jax.experimental import pallas as pl
from jax.experimental.pallas import tpu as pltpu

B, D, H, SK, DH, F = 4, 448, 16, 16384, 256, 1792
F32, BF16 = jnp.float32, jnp.bfloat16
NT_DIMS = (((1,), (1,)), ((), ()))


def _ln(x):
    m = jnp.mean(x, axis=-1, keepdims=True)
    xc = x - m
    v = jnp.mean(xc * xc, axis=-1, keepdims=True)
    return xc / jnp.sqrt(v + 1e-5)


def _silu(x):
    return x * (1.0 / (1.0 + jnp.exp(-x)))


def _make(CK=2048, NBUF=4, SUB=96, WSUB=32, ffn_last=True, wo_last=False, KS=None, VS=None):
    NC = SK // CK
    NU = B * H
    NT = NU * NC
    def pieces(szs):
        if szs is None:
            szs = [SUB] * (CK // SUB) + ([CK % SUB] if CK % SUB else [])
        assert sum(szs) == CK
        out, r = [], 0
        for n in szs:
            out.append((r, n)); r += n
        return out
    KP, VP = pieces(KS), pieces(VS)

    def kernel(x_hbm, k_hbm, v_hbm, wq_hbm, wot_hbm, wr_hbm, wg_hbm, wu_hbm, wdt_hbm, c_hbm, wmod_hbm, o_ref,
               kbuf, vbuf, ksem, vsem, wq_v, wot_v, wg_v, wu_v, wdt_v, wmod_v, x_v, c_v, wr_v, wsem, q_scr):
        def start(t, slot):
            base = t * CK
            for j in range(max(len(KP), len(VP))):
                if j < len(KP):
                    r, n = KP[j]
                    pltpu.make_async_copy(k_hbm.at[pl.ds(base + r, n)], kbuf.at[slot, pl.ds(r, n)], ksem.at[slot]).start(priority=0)
                if j < len(VP):
                    r, n = VP[j]
                    pltpu.make_async_copy(v_hbm.at[pl.ds(base + r, n)], vbuf.at[slot, pl.ds(r, n)], vsem.at[slot]).start(priority=1)

        def wait_k(slot):
            pltpu.make_async_copy(kbuf.at[slot], kbuf.at[slot], ksem.at[slot]).wait()

        def wait_v(slot):
            pltpu.make_async_copy(vbuf.at[slot], vbuf.at[slot], vsem.at[slot]).wait()

        W = dict(x=(x_hbm, x_v, 0), c=(c_hbm, c_v, 1), wr=(wr_hbm, wr_v, 2), wmod=(wmod_hbm, wmod_v, 3), wq=(wq_hbm, wq_v, 4),
                 wo=(wot_hbm, wot_v, 5), wg=(wg_hbm, wg_v, 6), wu=(wu_hbm, wu_v, 7), wd=(wdt_hbm, wdt_v, 8))

        def wstart(name):
            s, d, i = W[name]
            if len(s.shape) == 2 and s.shape[0] == D:
                for j in range(D // WSUB):
                    pltpu.make_async_copy(s.at[pl.ds(j * WSUB, WSUB)], d.at[pl.ds(j * WSUB, WSUB)], wsem.at[i]).start(priority=j % 2)
            else:
                pltpu.make_async_copy(s, d, wsem.at[i]).start()

        def wwait(name):
            s, d, i = W[name]
            pltpu.make_async_copy(d, d, wsem.at[i]).wait()

        for n in ("x", "c", "wr", "wmod", "wq"):
            wstart(n)
        for j in range(NBUF - 1):
            start(j, j)
        if not wo_last:
            wstart("wo")
        if not ffn_last:
            wstart("wg"); wstart("wu"); wstart("wd")

        wwait("x"); wwait("c"); wwait("wr")
        zpad = jnp.zeros((8 - B, D), F32)
        x8 = jnp.concatenate([x_v[...].astype(F32), zpad], axis=0)
        c8 = jnp.concatenate([c_v[...].astype(F32), zpad], axis=0)
        sc = _silu(c8).astype(BF16)
        ln1 = _ln(x8)
        wwait("wmod")
        mod = jnp.dot(sc, wmod_v[...], preferred_element_type=F32)
        sa, ca, ga, sb, cb, gb = [mod[:, i * D:(i + 1) * D] for i in range(6)]
        h1 = (ln1 * (1.0 + ca) + sa).astype(BF16)
        wwait("wq")
        q = jnp.dot(h1, wq_v[...], preferred_element_type=F32).astype(BF16).astype(F32) * (DH ** -0.5)
        for h in range(H):
            q_scr[h] = q[:, h * DH:(h + 1) * DH]
        if not wo_last:
            wwait("wo")
        row = jax.lax.broadcasted_iota(jnp.int32, (8, DH), 0)

        def attend(b, h):
            u = b * H + h
            qb = jnp.broadcast_to(q_scr[h, pl.ds(b, 1), :], (8, DH)).astype(BF16)

            def step(c, carry):
                m, l, acc = carry
                t = u * NC + c
                slot = t % NBUF
                nxt = t + NBUF - 1

                @pl.when(nxt < NT)
                def _():
                    start(nxt, nxt % NBUF)

                if ffn_last:
                    @pl.when(nxt == NT - 1)
                    def _():
                        wstart("wg"); wstart("wu"); wstart("wd")
                wait_k(slot)
                wait_v(slot)
                s = jax.lax.dot_general(qb, kbuf[slot], NT_DIMS, preferred_element_type=F32)
                m_new = jnp.maximum(m, jnp.max(s, axis=1, keepdims=True))
                alpha = jnp.exp(m - m_new)
                p = jnp.exp(s - m_new)
                l = alpha * l + jnp.sum(p, axis=1, keepdims=True)
                acc = alpha * acc + jnp.dot(p.astype(BF16), vbuf[slot], preferred_element_type=F32)
                return m_new, l, acc

            m, l, acc = jax.lax.fori_loop(0, NC, step, (jnp.full((8, 1), -jnp.inf, F32), jnp.zeros((8, 1), F32), jnp.zeros((8, DH), F32)))
            return jnp.where(row == b, acc / l, 0.0).astype(BF16)

        attn = jnp.zeros((8, D), F32)

        def bloop(b, attn):
            for h in range(H):
                o = attend(b, h)
                attn = attn + jax.lax.dot_general(o, wot_v[:, h * DH:(h + 1) * DH], NT_DIMS, preferred_element_type=F32)
            return attn
        attn = jax.lax.fori_loop(0, B, bloop, attn)

        x1 = x8 + ga * attn
        h2 = _ln(x1) * (1.0 + cb) + sb
        h2b = h2.astype(BF16)
        r = jnp.sum(h2b.astype(F32) * wr_v[...].astype(F32).reshape(1, D), axis=-1, keepdims=True)
        rs = 1.0 / (1.0 + jnp.exp(-r))
        wwait("wg")
        g = jnp.dot(h2b, wg_v[...], preferred_element_type=F32)
        wwait("wu")
        up = jnp.dot(h2b, wu_v[...], preferred_element_type=F32)
        a = (_silu(g) * up).astype(BF16)
        wwait("wd")
        y = jax.lax.dot_general(a, wdt_v[...], NT_DIMS, preferred_element_type=F32) * rs
        out = x1 + gb * (h2 + (h2 * 0.0 + y))
        o_ref[...] = out[0:B].astype(BF16)

    hbm = pl.BlockSpec(memory_space=pltpu.HBM)
    f = pl.pallas_call(
        kernel,
        out_shape=jax.ShapeDtypeStruct((B, D), BF16),
        in_specs=[hbm] * 11,
        out_specs=pl.BlockSpec(memory_space=pltpu.VMEM),
        scratch_shapes=[
            pltpu.VMEM((NBUF, CK, DH), BF16), pltpu.VMEM((NBUF, CK, DH), BF16),
            pltpu.SemaphoreType.DMA((NBUF,)), pltpu.SemaphoreType.DMA((NBUF,)),
            pltpu.VMEM((D, H * DH), BF16), pltpu.VMEM((D, H * DH), BF16),
            pltpu.VMEM((D, F), BF16), pltpu.VMEM((D, F), BF16), pltpu.VMEM((D, F), BF16),
            pltpu.VMEM((D, 6 * D), BF16), pltpu.VMEM((B, D), BF16), pltpu.VMEM((B, D), BF16), pltpu.VMEM((D,), BF16),
            pltpu.SemaphoreType.DMA((9,)),
            pltpu.VMEM((H, 8, DH), F32),
        ],
        compiler_params=pltpu.CompilerParams(vmem_limit_bytes=100 * 1024 * 1024),
    )

    def run(A_x, A_k_cache, A_v_cache, A_wq, A_wo, B_x, B_w_r, B_w_gate, B_w_up, B_w_down, c, w_mod):
        out = f(A_x.reshape(B, D), A_k_cache.reshape(B * H * SK, DH), A_v_cache.reshape(B * H * SK, DH), A_wq, A_wo.T, B_w_r, B_w_gate, B_w_up, B_w_down.T, c, w_mod)
        return out.reshape(B, 1, D)
    return run


@jax.jit
def pallas_adaLN_cond__mha_block_cached__moe_arch_mod__decode_kernel(
    A_x, A_k_cache, A_v_cache, A_wq, A_wo, B_x, B_w_r, B_w_gate, B_w_up, B_w_down, c, w_mod,
):
    return _make()(A_x, A_k_cache, A_v_cache, A_wq, A_wo, B_x, B_w_r, B_w_gate, B_w_up, B_w_down, c, w_mod)
```
